```python
import os as _os
_os.environ.setdefault('JAX_PLATFORMS', 'cpu')
import jax
import jax.numpy as jnp

def _softmax(x, axis=-1):
    return jax.nn.softmax(x, axis=axis)

def _gelu(x):
    return jax.nn.gelu(x, approximate=True)

def _silu(x):
    return jax.nn.silu(x)

def _sigmoid(x):
    return jax.nn.sigmoid(x)

def _layernorm(x, axis=-1, eps=1e-05):
    m = jnp.mean(x, axis=axis, keepdims=True)
    v = jnp.var(x, axis=axis, keepdims=True)
    return (x - m) / jnp.sqrt(v + eps)

def _scatter_add(tgt, idx, src, axis=0):
    return tgt.at[idx].add(src)

def _segment_sum(src, seg, n):
    return jax.ops.segment_sum(src, seg, n)

class _Rng:

    def __init__(self, key):
        self._k = key

    def _next(self):
        self._k, sub = jax.random.split(self._k)
        return sub

    def normal(self, shape):
        return jax.random.normal(self._next(), shape, dtype=jnp.bfloat16)

    def randint(self, lo, hi, shape):
        return jax.random.randint(self._next(), shape, lo, hi, dtype=jnp.int32)

    def uniform(self, shape, lo=0.0, hi=1.0):
        return jax.random.uniform(self._next(), shape, jnp.bfloat16, lo, hi)

    def permutation(self, n):
        return jax.random.permutation(self._next(), n)
kernel_name = 'gated_mix__memory_aug_recurrent_mem_tr__glu_gated_geglu__prompt'

def setup_inputs():
    _rng = _Rng(jax.random.key(int.from_bytes(__import__("os").urandom(4), "little")))
    _w = lambda a: (lambda t: t.astype(jnp.bfloat16) if jnp.issubdtype(t.dtype, jnp.floating) else t)(jnp.asarray(a))

    def _A_setup():
        B, S, Dm = (1, 2048, 640)
        H, Dh = (32, 128)
        M, seg = (8, 32)
        seg = min(seg, S)
        S = S // seg * seg
        return {'x': _w((lambda *s: _rng.normal(s) * 0.05)(B, S, Dm)), 'mem0': _w((lambda *s: _rng.normal(s) * 0.4)(B, M, Dm)), 'Wq': _w((lambda *s: _rng.normal(s) * 3.2)(Dm, H, Dh) * Dm ** (-0.5)), 'Wk': _w((lambda *s: _rng.normal(s) * 3.2)(Dm, H, Dh) * Dm ** (-0.5)), 'Wv': _w((lambda *s: _rng.normal(s) * 0.4)(Dm, H, Dh) * Dm ** (-0.5)), 'Wo': _w((lambda *s: _rng.normal(s) * 0.4)(H, Dh, Dm) * (H * Dh) ** (-0.5)), 'seg_len': seg}
    _A_in = _A_setup()

    def _B_setup():
        B, S, Dm, Df = (1, 2048, 640, 1728)
        return {'x': _w((lambda *s: _rng.normal(s) * 0.05)(B, S, Dm)), 'w_gate': _w((lambda *s: _rng.normal(s) * 1.6)(Dm, Df) * Dm ** (-0.5)), 'w_up': _w((lambda *s: _rng.normal(s) * 1.6)(Dm, Df) * Dm ** (-0.5)), 'w_down': _w((lambda *s: _rng.normal(s) * 1.6)(Df, Dm) * Df ** (-0.5))}
    _B_in = _B_setup()
    return {'A_x': _A_in['x'], 'A_mem0': _A_in['mem0'], 'A_Wq': _A_in['Wq'], 'A_Wk': _A_in['Wk'], 'A_Wv': _A_in['Wv'], 'A_Wo': _A_in['Wo'], 'A_seg_len': _A_in['seg_len'], 'B_x': _B_in['x'], 'B_w_gate': _B_in['w_gate'], 'B_w_up': _B_in['w_up'], 'B_w_down': _B_in['w_down'], 'gate_w': _w((lambda *s: _rng.normal(s) * 0.05)(640) * 16.0)}

def reference(A_x, A_mem0, A_Wq, A_Wk, A_Wv, A_Wo, A_seg_len, B_x, B_w_gate, B_w_up, B_w_down, gate_w):

    def _A_ref(x, mem0, Wq, Wk, Wv, Wo, seg_len):
        B, S, Dm = x.shape
        H, Dh = (Wq.shape[1], Wq.shape[2])
        M = mem0.shape[1]
        scale = Dh ** (-0.5)
        n_seg = S // seg_len
        L = M + seg_len
        idx = jnp.arange(L)
        mask = (idx[:, None] < M) | (idx[:, None] >= idx[None, :])
        mem = mem0
        outs = []
        for s in range(n_seg):
            xs = x[:, s * seg_len:(s + 1) * seg_len, :].copy()
            h = jnp.concatenate([mem, xs], axis=1)
            q = jnp.einsum('btd,dhe->bhte', h, Wq)
            k = jnp.einsum('btd,dhe->bhte', h, Wk)
            v = jnp.einsum('btd,dhe->bhte', h, Wv)
            scores = jnp.einsum('bhqe,bhke->bhqk', q, k) * scale
            scores = jnp.where(mask[None, None], scores, -1000000000.0)
            p = _softmax(scores, axis=-1)
            o = jnp.einsum('bhqk,bhke->bhqe', p, v)
            o = jnp.einsum('bhte,hed->btd', o, Wo)
            mem = o[:, :M, :].copy()
            outs.append(o[:, M:, :])
        return jnp.concatenate(outs, axis=1)

    def _B_ref(x, w_gate, w_up, w_down):
        g = jnp.einsum('bsd,df->bsf', x, w_gate)
        u = jnp.einsum('bsd,df->bsf', x, w_up)
        h = _gelu(g) * u
        return jnp.einsum('bsf,fd->bsd', h, w_down)
    x = A_x
    g = _sigmoid((x * gate_w).sum(-1, keepdims=True))
    a = _A_ref(x, A_mem0, A_Wq, A_Wk, A_Wv, A_Wo, A_seg_len)
    b = _B_ref(x, B_w_gate, B_w_up, B_w_down)
    return g * a + (1 - g) * b
```

```python
import functools

import jax
import jax.numpy as jnp
import jax.experimental.pallas as pl
import jax.experimental.pallas.tpu as pltpu

F32 = jnp.float32
BF16 = jnp.bfloat16
_NN = (((1,), (0,)), ((), ()))
_NT = (((1,), (1,)), ((), ()))


def _dot(a, b, dims=_NN):
    return jax.lax.dot_general(a, b, dims, preferred_element_type=F32)


def _rnd(a):
    return a.astype(BF16).astype(F32)


def _relayout(raw_ref, dst_ref, n_heads, t):
    hp = n_heads // 2
    wu = raw_ref.bitcast(jnp.uint32)
    ou = dst_ref.bitcast(jnp.uint32)
    wv = wu.at[pl.ds(pl.multiple_of(t * (16 * hp), 16 * hp), 16 * hp), :]
    ob = pl.multiple_of(t * 8, 8)
    for i in range(hp):
        a = wv[pl.ds(i, 8, stride=2 * hp), :]
        b = wv[pl.ds(hp + i, 8, stride=2 * hp), :]
        ou[pl.ds(ob, 8), (2 * i) * 128:(2 * i + 1) * 128] = (a & 0xFFFF) | (b << 16)
        ou[pl.ds(ob, 8), (2 * i + 1) * 128:(2 * i + 2) * 128] = (a >> 16) | ((b >> 16) << 16)


def _kernel(x_hbm, mem_hbm, wq_hbm, wk_hbm, wv_hbm, wo_hbm, wg_hbm, wu_hbm, wd_hbm, gw_hbm,
            out_hbm,
            x_v, mem_v, gw_v, wg_v, wu_v, wd_v, rq, rk, rv, wq_v, wk_v, wv_v, wo_v, b_v, out_v,
            sems, osem, *, S, M, seg, H, G, FC):
    Dh = 128
    srcs = (x_hbm, wg_hbm, wu_hbm, wd_hbm, gw_hbm, mem_hbm, wq_hbm, wk_hbm, wv_hbm, wo_hbm)
    dsts = (x_v, wg_v, wu_v, wd_v, gw_v, mem_v, rq, rk, rv, wo_v)
    cps = [pltpu.make_async_copy(s_, d_, sems.at[i]) for i, (s_, d_) in enumerate(zip(srcs, dsts))]
    for c in cps:
        c.start()
    for c in cps[:6]:
        c.wait()

    def ffn(c, carry):
        r0 = pl.multiple_of(c * FC, FC)
        xc = x_v[pl.ds(r0, FC), :]
        g = _dot(xc, wg_v[...])
        u = _dot(xc, wu_v[...])
        hh = (jax.nn.gelu(g, approximate=True) * u).astype(BF16)
        b = _dot(hh, wd_v[...])
        gate = jax.nn.sigmoid(jnp.sum(xc.astype(F32) * gw_v[...].astype(F32), axis=-1, keepdims=True))
        b_v[pl.ds(r0, FC), :] = (1.0 - gate) * b
        return carry

    jax.lax.fori_loop(0, S // FC, ffn, 0)

    for c in cps[6:]:
        c.wait()

    def rel(t, carry):
        _relayout(rq, wq_v, H, t)
        _relayout(rk, wk_v, H, t)
        _relayout(rv, wv_v, H, t)
        return carry

    jax.lax.fori_loop(0, wq_v.shape[0] // 16, rel, 0)

    L = M + seg
    scale = Dh ** -0.5
    ri = jax.lax.broadcasted_iota(jnp.int32, (L, L), 0)
    ci = jax.lax.broadcasted_iota(jnp.int32, (L, L), 1)
    mask = (ri < M) | (ri >= ci)

    def step(s, mem):
        r0 = pl.multiple_of(s * seg, seg)
        xs = x_v[pl.ds(r0, seg), :].astype(F32)
        h = jnp.concatenate([mem, xs], axis=0)
        acc = None
        for gi in range(H // G):
            cs = slice(gi * G * Dh, (gi + 1) * G * Dh)
            q = _rnd(_dot(h, wq_v[:, cs]))
            k = _dot(h, wk_v[:, cs]).astype(BF16)
            v = _dot(h, wv_v[:, cs]).astype(BF16)
            os_ = []
            for j in range(G):
                hs = slice(j * Dh, (j + 1) * Dh)
                sc = _dot(q[:, hs], k[:, hs], _NT) * scale
                sc = jnp.where(mask, sc, -1000000000.0)
                e = jnp.exp(sc - jnp.max(sc, axis=-1, keepdims=True))
                p = _rnd(e / jnp.sum(e, axis=-1, keepdims=True))
                os_.append(_dot(p, v[:, hs]))
            o = _rnd(jnp.concatenate(os_, axis=1))
            part = _dot(o, wo_v[cs, :])
            acc = part if acc is None else acc + part
        gate = jax.nn.sigmoid(jnp.sum(xs * gw_v[...].astype(F32), axis=-1, keepdims=True))
        out_v[pl.ds(r0, seg), :] = (gate * acc[M:] + b_v[pl.ds(r0, seg), :]).astype(BF16)
        pltpu.make_async_copy(out_v.at[pl.ds(r0, seg), :], out_hbm.at[pl.ds(r0, seg), :], osem).start()
        return _rnd(acc[:M])

    jax.lax.fori_loop(0, S // seg, step, mem_v[...].astype(F32))
    pltpu.make_async_copy(out_v, out_v, osem).wait()


@functools.partial(jax.jit, static_argnames=("A_seg_len",))
def pallas_gated_mix__memory_aug_recurrent_mem_tr__glu_gated_geglu__prompt_kernel(
    A_x, A_mem0, A_Wq, A_Wk, A_Wv, A_Wo, A_seg_len, B_x, B_w_gate, B_w_up, B_w_down, gate_w,
):
    del B_x
    B, S, Dm = A_x.shape
    _, H, Dh = A_Wq.shape
    M = A_mem0.shape[1]
    Df = B_w_gate.shape[1]
    seg = int(A_seg_len)
    assert B == 1 and Dh == 128 and S % seg == 0
    kern = functools.partial(_kernel, S=S, M=M, seg=seg, H=H, G=4, FC=256)
    vm = pltpu.VMEM
    out = pl.pallas_call(
        kern,
        out_shape=jax.ShapeDtypeStruct((S, Dm), BF16),
        in_specs=[pl.BlockSpec(memory_space=pl.ANY)] * 10,
        out_specs=pl.BlockSpec(memory_space=pl.ANY),
        scratch_shapes=[
            vm((S, Dm), BF16), vm((M, Dm), BF16), vm((1, Dm), BF16),
            vm((Dm, Df), BF16), vm((Dm, Df), BF16), vm((Df, Dm), BF16),
            vm((Dm * H, Dh), BF16), vm((Dm * H, Dh), BF16), vm((Dm * H, Dh), BF16),
            vm((Dm, H * Dh), BF16), vm((Dm, H * Dh), BF16), vm((Dm, H * Dh), BF16),
            vm((H * Dh, Dm), BF16), vm((S, Dm), F32), vm((S, Dm), BF16),
            pltpu.SemaphoreType.DMA((10,)), pltpu.SemaphoreType.DMA(()),
        ],
        compiler_params=pltpu.CompilerParams(vmem_limit_bytes=100 * 2**20),
    )(A_x.reshape(S, Dm), A_mem0.reshape(M, Dm),
      A_Wq.reshape(Dm * H, Dh), A_Wk.reshape(Dm * H, Dh), A_Wv.reshape(Dm * H, Dh),
      A_Wo.reshape(H * Dh, Dm), B_w_gate, B_w_up, B_w_down, gate_w.reshape(1, Dm))
    return out.reshape(B, S, Dm)
```

```python
import functools

import jax
import jax.numpy as jnp
import jax.experimental.pallas as pl
import jax.experimental.pallas.tpu as pltpu

F32 = jnp.float32
BF16 = jnp.bfloat16
_NN = (((1,), (0,)), ((), ()))
_NT = (((1,), (1,)), ((), ()))


def _dot(a, b, dims=_NN):
    return jax.lax.dot_general(a, b, dims, preferred_element_type=F32)


def _rnd(a):
    return a.astype(BF16).astype(F32)


def _bf(u):
    return pltpu.bitcast(u, BF16)


def _relayout(raw_ref, dst_ref, n_heads, t):
    hp = n_heads // 2
    wu = raw_ref
    ou = dst_ref
    wv = wu.at[pl.ds(pl.multiple_of(t * (16 * hp), 16 * hp), 16 * hp), :]
    ob = pl.multiple_of(t * 8, 8)
    for i in range(hp):
        a = wv[pl.ds(i, 8, stride=2 * hp), :]
        b = wv[pl.ds(hp + i, 8, stride=2 * hp), :]
        ou[pl.ds(ob, 8), (2 * i) * 128:(2 * i + 1) * 128] = (a & 0xFFFF) | (b << 16)
        ou[pl.ds(ob, 8), (2 * i + 1) * 128:(2 * i + 2) * 128] = (a >> 16) | ((b >> 16) << 16)


def _kernel(x_hbm, mem_hbm, wq_hbm, wk_hbm, wv_hbm, wo_hbm, wg_hbm, wu_hbm, wd_hbm, gw_hbm,
            out_hbm,
            x_v, mem_v, gw_v, wg_r, wu_r, wd_r, wg_v, wu_v, wd_v, ra, wa_v, ro, wo_v, b_v, out_v,
            sems, osem, *, S, M, seg, H, G, FC):
    Dh = 128
    RN = ra.shape[0] // 3
    rq, rk, rv = (ra.at[m * RN:(m + 1) * RN] for m in range(3))
    srcs = (x_hbm.at[0:2 * FC], wg_hbm, wu_hbm, wd_hbm, gw_hbm, mem_hbm,
            wq_hbm.bitcast(jnp.uint32), wk_hbm.bitcast(jnp.uint32), wv_hbm.bitcast(jnp.uint32), wo_hbm,
            x_hbm.at[2 * FC:])
    dsts = (x_v.at[0:2 * FC], wg_r, wu_r, wd_r, gw_v, mem_v, rq, rk, rv, ro, x_v.at[2 * FC:])
    cps = [pltpu.make_async_copy(s_, d_, sems.at[i]) for i, (s_, d_) in enumerate(zip(srcs, dsts))]
    for i in (1, 2, 3, 0, 4, 5, 10, 6):
        cps[i].start()

    Df = wd_r.shape[0]
    Dp = 2 * wd_v.shape[0]
    FH = Dp // 2
    for src, dst, cp in ((wg_r, wg_v, cps[1]), (wu_r, wu_v, cps[2])):
        cp.wait()
        for j in range(Dp // 128):
            n = min(128, Df - j * 128)
            blk = src[j * 128:j * 128 + n, :]
            if n < 128:
                blk = jnp.concatenate([blk, jnp.zeros((128 - n, blk.shape[1]), BF16)], axis=0)
            jj = j % (FH // 128)
            dst[j // (FH // 128), :, jj * 128:(jj + 1) * 128] = pltpu.bitcast(blk.T, jnp.uint32)
    cps[3].wait()
    wd_v[0:Df // 2, :] = pltpu.bitcast(wd_r[...], jnp.uint32)
    if Dp > Df:
        wd_v[Df // 2:, :] = jnp.zeros(((Dp - Df) // 2, wd_v.shape[1]), jnp.uint32)

    n_bulk = S // 2 // FC
    per = wa_v.shape[0] // 8 // (n_bulk - 2)

    def ffn(c, with_rel):
        r0 = pl.multiple_of((c + 2) * FC, FC)
        xc = x_v[pl.ds(r0, FC), :]
        b = None
        for hf in range(2):
            g = _dot(xc, _bf(wg_v[hf]))
            u = _dot(xc, _bf(wu_v[hf]))
            hh = (jax.nn.gelu(g, approximate=True) * u).astype(BF16)
            t = _dot(hh, _bf(wd_v[hf * FH // 2:(hf + 1) * FH // 2, :]))
            b = t if b is None else b + t
        b_v[pl.ds(r0, FC), :] = b
        if with_rel:
            for t in range(per):
                _relayout(ra, wa_v, H, c * per + t)

    for i in (0, 4, 5):
        cps[i].wait()
    jax.lax.fori_loop(0, 2, lambda c, z: ffn(c - 2, False), None)
    cps[10].wait()

    def loop2(c, carry):
        for m in range(3):
            @pl.when(c == m * (n_bulk - 2) // 3)
            def _():
                cps[6 + m].wait()
                cps[7 + m].start()
        ffn(c, True)
        return carry

    jax.lax.fori_loop(0, n_bulk - 2, loop2, 0)
    cps[9].wait()

    def relo(t, carry):
        blk = ro[pl.ds(pl.multiple_of(t * 128, 128), 128), :]
        wo_v[pl.ds(pl.multiple_of(t * 64, 64), 64), :] = pltpu.bitcast(blk, jnp.uint32)
        return carry

    jax.lax.fori_loop(0, ro.shape[0] // 128, relo, 0)
    DH2 = wa_v.shape[0] // 3
    wq_v, wk_v, wv_v = (wa_v.at[m * DH2:(m + 1) * DH2] for m in range(3))

    L = M + seg
    scale = Dh ** -0.5
    ri = jax.lax.broadcasted_iota(jnp.int32, (L, L), 0)
    ci = jax.lax.broadcasted_iota(jnp.int32, (L, L), 1)
    mask = (ri < M) | (ri >= ci)

    def step(p_, half, mem, fb0):
        s = 2 * p_ + half
        r0 = pl.multiple_of(s * seg, seg)
        xs = x_v[pl.ds(r0, seg), :].astype(F32)
        h = jnp.concatenate([mem, xs], axis=0)
        NG = H // G
        GW = G * Dh
        pq = lambda g: _rnd(_dot(h, _bf(wq_v[:, g * GW:(g + 1) * GW])))
        pk = lambda g: _dot(h, _bf(wk_v[:, g * GW:(g + 1) * GW])).astype(BF16)
        pv = lambda g: _dot(h, _bf(wv_v[:, g * GW:(g + 1) * GW])).astype(BF16)
        hsl = [slice(j * Dh, (j + 1) * Dh) for j in range(G)]
        acc = None
        q, k, v = pq(0), pk(0), pv(0)
        for gi in range(NG):
            nxt = gi + 1 < NG
            scs = [_dot(q[:, hs], k[:, hs], _NT) for hs in hsl]
            if nxt:
                k = pk(gi + 1)
                q = pq(gi + 1)
            else:
                f0 = half * (FH // 2)
                rf = pl.multiple_of(S // 2 + p_ * seg, seg)
                xf = x_v[pl.ds(rf, seg), :]
                fg = _dot(xf, _bf(wg_v[half]))
                fu0 = _dot(xf, _bf(wu_v[half, :, 0:512]))
            ps = []
            for sc in scs:
                sc = jnp.where(mask, sc * scale, -1000000000.0)
                e = jnp.exp(sc - jnp.max(sc, axis=-1, keepdims=True))
                ps.append(_rnd(e * (1.0 / jnp.sum(e, axis=-1, keepdims=True))))
            o = _rnd(jnp.concatenate([_dot(p, v[:, hs]) for p, hs in zip(ps, hsl)], axis=1))
            if nxt:
                v = pv(gi + 1)
            else:
                fu1 = _dot(xf, _bf(wu_v[half, :, 512:FH]))
            part = _dot(o, _bf(wo_v[gi * GW // 2:(gi + 1) * GW // 2, :]))
            if not nxt:
                fu = jnp.concatenate([fu0, fu1], axis=1)
                hh = (jax.nn.gelu(fg, approximate=True) * fu).astype(BF16)
                fb = _dot(hh, _bf(wd_v[pl.ds(f0, FH // 2), :]))
                if half:
                    b_v[pl.ds(rf, seg), :] = fb + fb0
            acc = part if acc is None else acc + part
        gate = jax.nn.sigmoid(jnp.sum(xs * gw_v[...].astype(F32), axis=-1, keepdims=True))
        out_v[pl.ds(r0, seg), :] = (gate * acc[M:] + (1.0 - gate) * b_v[pl.ds(r0, seg), :]).astype(BF16)
        pltpu.make_async_copy(out_v.at[pl.ds(r0, seg), :], out_hbm.at[pl.ds(r0, seg), :], osem).start()
        return _rnd(acc[:M]), fb

    def pair(p_, mem):
        mem, fb0 = step(p_, 0, mem, None)
        return step(p_, 1, mem, fb0)[0]

    jax.lax.fori_loop(0, S // seg // 2, pair, mem_v[...].astype(F32))
    pltpu.make_async_copy(out_v, out_v, osem).wait()


@functools.partial(jax.jit, static_argnames=("A_seg_len",))
def pallas_gated_mix__memory_aug_recurrent_mem_tr__glu_gated_geglu__prompt_kernel(
    A_x, A_mem0, A_Wq, A_Wk, A_Wv, A_Wo, A_seg_len, B_x, B_w_gate, B_w_up, B_w_down, gate_w,
):
    del B_x
    B, S, Dm = A_x.shape
    _, H, Dh = A_Wq.shape
    M = A_mem0.shape[1]
    Df = B_w_gate.shape[1]
    seg = int(A_seg_len)
    assert B == 1 and Dh == 128 and S % seg == 0
    kern = functools.partial(_kernel, S=S, M=M, seg=seg, H=H, G=4, FC=128)
    vm = pltpu.VMEM
    Dp = -(-Df // 256) * 256
    out = pl.pallas_call(
        kern,
        out_shape=jax.ShapeDtypeStruct((S, Dm), BF16),
        in_specs=[pl.BlockSpec(memory_space=pl.ANY)] * 10,
        out_specs=pl.BlockSpec(memory_space=pl.ANY),
        scratch_shapes=[
            vm((S, Dm), BF16), vm((M, Dm), BF16), vm((1, Dm), BF16),
            vm((Df, Dm), BF16), vm((Df, Dm), BF16), vm((Df, Dm), BF16),
            vm((2, Dm // 2, Dp // 2), jnp.uint32), vm((2, Dm // 2, Dp // 2), jnp.uint32), vm((Dp // 2, Dm), jnp.uint32),
            vm((3 * Dm * H // 2, Dh), jnp.uint32),
            vm((3 * Dm // 2, H * Dh), jnp.uint32),
            vm((H * Dh, Dm), BF16), vm((H * Dh // 2, Dm), jnp.uint32), vm((S, Dm), F32), vm((S, Dm), BF16),
            pltpu.SemaphoreType.DMA((11,)), pltpu.SemaphoreType.DMA(()),
        ],
        compiler_params=pltpu.CompilerParams(vmem_limit_bytes=100 * 2**20),
    )(A_x.reshape(S, Dm), A_mem0.reshape(M, Dm),
      A_Wq.reshape(Dm * H, Dh), A_Wk.reshape(Dm * H, Dh), A_Wv.reshape(Dm * H, Dh),
      A_Wo.reshape(H * Dh, Dm), B_w_gate.T, B_w_up.T, B_w_down, gate_w.reshape(1, Dm))
    return out.reshape(B, S, Dm)
```
